```python
import os as _os
_os.environ.setdefault("JAX_PLATFORMS", "cpu")
import jax
import jax.numpy as jnp

def _softmax(x, axis=-1):
    return jax.nn.softmax(x, axis=axis)
def _gelu(x):
    return jax.nn.gelu(x, approximate=True)
def _silu(x):
    return jax.nn.silu(x)
def _sigmoid(x):
    return jax.nn.sigmoid(x)
def _layernorm(x, axis=-1, eps=1e-5):
    m = jnp.mean(x, axis=axis, keepdims=True)
    v = jnp.var(x, axis=axis, keepdims=True)
    return (x - m) / jnp.sqrt(v + eps)
def _scatter_add(tgt, idx, src, axis=0):
    return tgt.at[idx].add(src)
def _segment_sum(src, seg, n):
    return jax.ops.segment_sum(src, seg, n)
class _Rng:
    def __init__(self, key):
        self._k = key
    def _next(self):
        self._k, sub = jax.random.split(self._k)
        return sub
    def normal(self, shape):
        return jax.random.normal(self._next(), shape, dtype=jnp.bfloat16)
    def randint(self, lo, hi, shape):
        return jax.random.randint(self._next(), shape, lo, hi, dtype=jnp.int32)
    def uniform(self, shape, lo=0.0, hi=1.0):
        return jax.random.uniform(self._next(), shape, jnp.bfloat16, lo, hi)
    def permutation(self, n):
        return jax.random.permutation(self._next(), n)


kernel_name = 'standalone__mha_softmax__near_ridge'

def setup_inputs():
    _rng = _Rng(jax.random.key(int.from_bytes(__import__("os").urandom(4), "little")))
    _w = (lambda a: (lambda t: t.astype(jnp.bfloat16) if jnp.issubdtype(t.dtype, jnp.floating) else t)(jnp.asarray(a)))
    B, H, Sq, Sk, D = 8, 16, 192, 1024, 256
    return {
        "q": _w((lambda *s: _rng.normal(s) * 0.4)(B, H, Sq, D)),
        "k": _w((lambda *s: _rng.normal(s) * 0.4)(B, H, Sk, D)),
        "v": _w((lambda *s: _rng.normal(s) * 0.05)(B, H, Sk, D)),
    }

def reference(q, k, v):
    scale = q.shape[-1] ** -0.5
    scores = jnp.einsum("bhqd,bhkd->bhqk", q, k) * scale
    p = _softmax(scores, axis=-1)
    return jnp.einsum("bhqk,bhkd->bhqd", p, v)
```

```python
import math

import jax
import jax.numpy as jnp
import jax.experimental.pallas as pl
import jax.experimental.pallas.tpu as pltpu

GROUP = 4
LOOKAHEAD = 2
READ_ROWS = 64
WRITE_STREAMS = 8
WRITE_ROWS = 32
WRITES_PER_HEAD = 8


def _attention_kernel(q_hbm, k_hbm, v_hbm, o_hbm, buf, out_buf, in_sems, out_sem):
    n_groups, _, sq, d = q_hbm.shape
    sk = k_hbm.shape[2]
    n_slots = buf.shape[0]
    heads_per_stream = n_groups * GROUP // WRITE_STREAMS
    n_writes = out_buf.shape[1] // WRITE_ROWS
    k_row, v_row, q_row = 0, sk, 2 * sk
    exp2_scale = d ** -0.5 * math.log2(math.e)

    def start_fetch(group, slot, turn):
        kv_pieces = sk // READ_ROWS // GROUP
        q_pieces = sq // READ_ROWS
        q_every = kv_pieces * GROUP // q_pieces
        for piece in range(kv_pieces):
            row = pl.multiple_of((turn * kv_pieces + piece) * READ_ROWS, READ_ROWS)
            for head in range(GROUP):
                for src, base, priority in ((k_hbm, k_row, 0), (v_hbm, v_row, 1)):
                    pltpu.make_async_copy(
                        src.at[group, head, pl.ds(row, READ_ROWS)],
                        buf.at[slot, head, pl.ds(base + row, READ_ROWS)],
                        in_sems.at[slot],
                    ).start(priority=priority)
                q_piece, phase = divmod(piece * GROUP + head, q_every)
                if phase == q_every // 2 and q_piece < q_pieces:
                    pltpu.make_async_copy(
                        q_hbm.at[group, turn, pl.ds(q_piece * READ_ROWS, READ_ROWS)],
                        buf.at[slot, turn,
                               pl.ds(q_row + q_piece * READ_ROWS, READ_ROWS)],
                        in_sems.at[slot],
                    ).start(priority=0)

    def wait_fetch(slot):
        pltpu.make_async_copy(buf.at[slot], buf.at[slot], in_sems.at[slot]).wait()

    def attend(group, slot, head):
        q = buf[slot, head, pl.ds(q_row, sq)]
        k = buf[slot, head, pl.ds(k_row, sk)]
        s = jax.lax.dot_general(q, k, (((1,), (1,)), ((), ())),
                                preferred_element_type=jnp.float32)
        m = jnp.max(s, axis=-1, keepdims=True)
        p = jnp.exp2((s - m) * exp2_scale)
        l = jnp.sum(p, axis=-1, keepdims=True)
        v = buf[slot, head, pl.ds(v_row, sk)]
        o = jnp.dot(p.astype(v.dtype), v, preferred_element_type=jnp.float32)
        o = o * (1.0 / l)
        index = group * GROUP + head
        row = pl.multiple_of((index % heads_per_stream) * sq, sq)
        out_buf[index // heads_per_stream, pl.ds(row, sq)] = o.astype(out_buf.dtype)

    def start_write(index):
        rows = pl.ds(pl.multiple_of(index * WRITE_ROWS, WRITE_ROWS), WRITE_ROWS)
        pltpu.make_async_copy(
            out_buf.at[:, rows], o_hbm.at[:, rows], out_sem.at[0]).start()

    @pl.loop(0, LOOKAHEAD * GROUP)
    def _(index):
        start_fetch(index // GROUP, index // GROUP, index % GROUP)

    @pl.loop(0, n_groups - LOOKAHEAD)
    def _(group):
        slot = group % n_slots
        wait_fetch(slot)

        @pl.loop(0, GROUP)
        def _(head):
            attend(group, slot, head)
            start_fetch(group + LOOKAHEAD, (group + LOOKAHEAD) % n_slots, head)

    @pl.loop(n_groups - LOOKAHEAD, n_groups)
    def _(group):
        slot = group % n_slots

        @pl.loop(0, GROUP)
        def _(head):
            done = (group - (n_groups - LOOKAHEAD)) * GROUP + head
            for offset in range(WRITES_PER_HEAD):
                start_write(done * WRITES_PER_HEAD + offset)

            @pl.when(head == 0)
            def _():
                wait_fetch(slot)

            attend(group, slot, head)

    @pl.loop(LOOKAHEAD * GROUP * WRITES_PER_HEAD, n_writes)
    def _(index):
        start_write(index)

    pltpu.make_async_copy(out_buf, o_hbm, out_sem.at[0]).wait()


@jax.jit
def pallas_standalone__mha_softmax__near_ridge_kernel(
    q: jax.Array,
    k: jax.Array,
    v: jax.Array,
):
    b, h, sq, d = q.shape
    sk = k.shape[2]
    n_heads = b * h
    n_groups = n_heads // GROUP
    n_slots = LOOKAHEAD + 1
    stream_rows = n_heads * sq // WRITE_STREAMS

    assert q.dtype == k.dtype == v.dtype
    assert n_heads % GROUP == 0 and n_heads % WRITE_STREAMS == 0
    assert sk % (READ_ROWS * GROUP) == 0 and sq % READ_ROWS == 0
    assert sq // READ_ROWS <= sk // READ_ROWS
    assert stream_rows % WRITE_ROWS == 0
    tail_heads = LOOKAHEAD * GROUP
    for done in range(tail_heads):
        last_row = (done + 1) * WRITES_PER_HEAD * WRITE_ROWS - 1
        assert last_row < stream_rows
        last_head = n_heads - n_heads // WRITE_STREAMS + last_row // sq
        assert last_head < n_heads - tail_heads + done

    hbm = pl.BlockSpec(memory_space=pl.ANY)
    out = pl.pallas_call(
        _attention_kernel,
        in_specs=[hbm, hbm, hbm],
        out_specs=hbm,
        out_shape=jax.ShapeDtypeStruct((WRITE_STREAMS, stream_rows, d), q.dtype),
        scratch_shapes=[
            pltpu.VMEM((n_slots, GROUP, 2 * sk + sq, d), q.dtype),
            pltpu.VMEM((WRITE_STREAMS, stream_rows, d), q.dtype),
            pltpu.SemaphoreType.DMA((n_slots,)),
            pltpu.SemaphoreType.DMA((1,)),
        ],
        compiler_params=pltpu.CompilerParams(
            vmem_limit_bytes=64 * 1024 * 1024),
        name="mha_softmax",
    )(
        q.reshape(n_groups, GROUP, sq, d),
        k.reshape(n_groups, GROUP, sk, d),
        v.reshape(n_groups, GROUP, sk, d),
    )
    return out.reshape(b, h, sq, d)
```

```python
import math

import jax
import jax.numpy as jnp
import jax.experimental.pallas as pl
import jax.experimental.pallas.tpu as pltpu

GROUP = 4
LOOKAHEAD = 2
READ_ROWS = 64
WRITE_STREAMS = 8
WRITE_ROWS = 32
WRITES_PER_HEAD = 10
WRITE_DELAY = 2


def _attention_kernel(q_hbm, k_hbm, v_hbm, o_hbm, buf, out_buf, in_sems, out_sem):
    n_groups, _, sq, d = q_hbm.shape
    sk = k_hbm.shape[2]
    n_slots = buf.shape[0]
    heads_per_stream = n_groups * GROUP // WRITE_STREAMS
    n_writes = out_buf.shape[1] // WRITE_ROWS
    k_row, v_row, q_row = 0, sk, 2 * sk
    exp2_scale = d ** -0.5 * math.log2(math.e)

    def start_fetch(group, slot, turn):
        kv_pieces = sk // READ_ROWS // GROUP
        q_pieces = sq // READ_ROWS
        q_every = kv_pieces * GROUP // q_pieces
        for piece in range(kv_pieces):
            row = pl.multiple_of((turn * kv_pieces + piece) * READ_ROWS, READ_ROWS)
            for head in range(GROUP):
                for src, base, priority in ((k_hbm, k_row, 0), (v_hbm, v_row, 1)):
                    pltpu.make_async_copy(
                        src.at[group, head, pl.ds(row, READ_ROWS)],
                        buf.at[slot, head, pl.ds(base + row, READ_ROWS)],
                        in_sems.at[slot],
                    ).start(priority=priority)
                q_piece, phase = divmod(piece * GROUP + head, q_every)
                if phase == q_every // 2 and q_piece < q_pieces:
                    pltpu.make_async_copy(
                        q_hbm.at[group, turn, pl.ds(q_piece * READ_ROWS, READ_ROWS)],
                        buf.at[slot, turn,
                               pl.ds(q_row + q_piece * READ_ROWS, READ_ROWS)],
                        in_sems.at[slot],
                    ).start(priority=0)

    def wait_fetch(slot):
        pltpu.make_async_copy(buf.at[slot], buf.at[slot], in_sems.at[slot]).wait()

    def attend(group, slot, head):
        q = buf[slot, head, pl.ds(q_row, sq)]
        k = buf[slot, head, pl.ds(k_row, sk)]
        s = jax.lax.dot_general(q, k, (((1,), (1,)), ((), ())),
                                preferred_element_type=jnp.float32)
        m = jnp.max(s, axis=-1, keepdims=True)
        p = jnp.exp2((s - m) * exp2_scale)
        l = jnp.sum(p, axis=-1, keepdims=True)
        v = buf[slot, head, pl.ds(v_row, sk)]
        o = jnp.dot(p.astype(v.dtype), v, preferred_element_type=jnp.float32)
        o = o * (1.0 / l)
        index = group * GROUP + head
        row = pl.multiple_of((index % heads_per_stream) * sq, sq)
        out_buf[index // heads_per_stream, pl.ds(row, sq)] = o.astype(out_buf.dtype)

    def start_write(index):
        rows = pl.ds(pl.multiple_of(index * WRITE_ROWS, WRITE_ROWS), WRITE_ROWS)
        pltpu.make_async_copy(
            out_buf.at[:, rows], o_hbm.at[:, rows], out_sem.at[0]).start()

    @pl.loop(0, LOOKAHEAD * GROUP)
    def _(index):
        start_fetch(index // GROUP, index // GROUP, index % GROUP)

    @pl.loop(0, n_groups - LOOKAHEAD)
    def _(group):
        slot = group % n_slots
        wait_fetch(slot)

        @pl.loop(0, GROUP)
        def _(head):
            attend(group, slot, head)
            start_fetch(group + LOOKAHEAD, (group + LOOKAHEAD) % n_slots, head)

    @pl.loop(n_groups - LOOKAHEAD, n_groups)
    def _(group):
        slot = group % n_slots

        @pl.loop(0, GROUP)
        def _(head):
            batch = (group - (n_groups - LOOKAHEAD)) * GROUP + head - WRITE_DELAY

            @pl.when(batch >= 0)
            def _():
                for offset in range(WRITES_PER_HEAD):
                    start_write(batch * WRITES_PER_HEAD + offset)

            @pl.when(head == 0)
            def _():
                wait_fetch(slot)

            attend(group, slot, head)

    @pl.loop((LOOKAHEAD * GROUP - WRITE_DELAY) * WRITES_PER_HEAD, n_writes)
    def _(index):
        start_write(index)

    pltpu.make_async_copy(out_buf, o_hbm, out_sem.at[0]).wait()


@jax.jit
def pallas_standalone__mha_softmax__near_ridge_kernel(
    q: jax.Array,
    k: jax.Array,
    v: jax.Array,
):
    b, h, sq, d = q.shape
    sk = k.shape[2]
    n_heads = b * h
    n_groups = n_heads // GROUP
    n_slots = LOOKAHEAD + 1
    stream_rows = n_heads * sq // WRITE_STREAMS

    assert q.dtype == k.dtype == v.dtype
    assert n_heads % GROUP == 0 and n_heads % WRITE_STREAMS == 0
    assert n_groups >= LOOKAHEAD
    assert sk % (READ_ROWS * GROUP) == 0 and sq % READ_ROWS == 0
    assert sq <= sk
    assert stream_rows % WRITE_ROWS == 0
    tail_heads = LOOKAHEAD * GROUP
    for done in range(WRITE_DELAY, tail_heads):
        last_row = (done - WRITE_DELAY + 1) * WRITES_PER_HEAD * WRITE_ROWS - 1
        assert last_row < stream_rows
        last_head = n_heads - n_heads // WRITE_STREAMS + last_row // sq
        assert last_head < n_heads - tail_heads + done

    hbm = pl.BlockSpec(memory_space=pl.ANY)
    out = pl.pallas_call(
        _attention_kernel,
        in_specs=[hbm, hbm, hbm],
        out_specs=hbm,
        out_shape=jax.ShapeDtypeStruct((WRITE_STREAMS, stream_rows, d), q.dtype),
        scratch_shapes=[
            pltpu.VMEM((n_slots, GROUP, 2 * sk + sq, d), q.dtype),
            pltpu.VMEM((WRITE_STREAMS, stream_rows, d), q.dtype),
            pltpu.SemaphoreType.DMA((n_slots,)),
            pltpu.SemaphoreType.DMA((1,)),
        ],
        compiler_params=pltpu.CompilerParams(
            vmem_limit_bytes=64 * 1024 * 1024),
        name="mha_softmax",
    )(
        q.reshape(n_groups, GROUP, sq, d),
        k.reshape(n_groups, GROUP, sk, d),
        v.reshape(n_groups, GROUP, sk, d),
    )
    return out.reshape(b, h, sq, d)
```
